```python
import os as _os
_os.environ.setdefault("JAX_PLATFORMS", "cpu")
import jax
import jax.numpy as jnp

def _softmax(x, axis=-1):
    return jax.nn.softmax(x, axis=axis)
def _gelu(x):
    return jax.nn.gelu(x, approximate=True)
def _silu(x):
    return jax.nn.silu(x)
def _sigmoid(x):
    return jax.nn.sigmoid(x)
def _layernorm(x, axis=-1, eps=1e-5):
    m = jnp.mean(x, axis=axis, keepdims=True)
    v = jnp.var(x, axis=axis, keepdims=True)
    return (x - m) / jnp.sqrt(v + eps)
def _scatter_add(tgt, idx, src, axis=0):
    return tgt.at[idx].add(src)
def _segment_sum(src, seg, n):
    return jax.ops.segment_sum(src, seg, n)
class _Rng:
    def __init__(self, key):
        self._k = key
    def _next(self):
        self._k, sub = jax.random.split(self._k)
        return sub
    def normal(self, shape):
        return jax.random.normal(self._next(), shape, dtype=jnp.bfloat16)
    def randint(self, lo, hi, shape):
        return jax.random.randint(self._next(), shape, lo, hi, dtype=jnp.int32)
    def uniform(self, shape, lo=0.0, hi=1.0):
        return jax.random.uniform(self._next(), shape, jnp.bfloat16, lo, hi)
    def permutation(self, n):
        return jax.random.permutation(self._next(), n)


kernel_name = 'standalone__gqa_block_cached__sampling'

def setup_inputs():
    _rng = _Rng(jax.random.key(int.from_bytes(__import__("os").urandom(4), "little")))
    _w = (lambda a: (lambda t: t.astype(jnp.bfloat16) if jnp.issubdtype(t.dtype, jnp.floating) else t)(jnp.asarray(a)))
    B, Sq, D = 32, 16, 1024
    Hq, Hkv, Sk, Dh = 32, 4, 2048, 128
    assert Hq % Hkv == 0, (Hq, Hkv)
    return {
        "x": _w((lambda *s: _rng.normal(s) * 0.8)(B, Sq, D)),
        "k_cache": _w((lambda *s: _rng.normal(s) * 0.8)(B, Hkv, Sk, Dh)),
        "v_cache": _w((lambda *s: _rng.normal(s) * 0.05)(B, Hkv, Sk, Dh)),
        "wq": _w((lambda *s: _rng.normal(s) * 0.8)(D, Hq * Dh) * (D ** -0.5)),
        "wo": _w((lambda *s: _rng.normal(s) * 0.05)(Hq * Dh, D) * ((Hq * Dh) ** -0.5)),
    }

def reference(x, k_cache, v_cache, wq, wo):
    B, Sq, D = x.shape
    Hq, Dh = 32, 128
    Hkv = k_cache.shape[1]
    rep = Hq // Hkv
    q = (lambda x, *d: x.transpose(*d))((x @ wq).reshape(B, Sq, Hq, Dh), 0, 2, 1, 3)
    k = jnp.repeat(k_cache, rep, axis=1)
    v = jnp.repeat(v_cache, rep, axis=1)
    scores = jnp.einsum("bhqd,bhkd->bhqk", q, k) * (Dh ** -0.5)
    p = _softmax(scores, axis=-1)
    o = jnp.einsum("bhqk,bhkd->bhqd", p, v)
    return (lambda x, *d: x.transpose(*d))(o, 0, 2, 1, 3).reshape(B, Sq, Hq * Dh) @ wo
```

```python
import functools

import jax
import jax.numpy as jnp
from jax import lax
import jax.experimental.pallas as pl
import jax.experimental.pallas.tpu as pltpu


@jax.jit
def pallas_standalone__gqa_block_cached__sampling_kernel(
    x: jax.Array,
    k_cache: jax.Array,
    v_cache: jax.Array,
    wq: jax.Array,
    wo: jax.Array,
):
    B, Sq, D = x.shape
    _, Hkv, Sk, Dh = k_cache.shape
    Hq = wq.shape[1] // Dh
    rep = Hq // Hkv
    M = B * Sq
    GW = rep * Dh
    scale = float(Dh) ** -0.5

    x2 = x.reshape(M, D)

    def kernel(x_ref, wq_ref, k_ref, v_ref, wo_ref, o_ref, q_scr, og_scr, acc_scr):
        g = pl.program_id(0)
        b = pl.program_id(1)

        @pl.when(b == 0)
        def _():
            q = jnp.dot(x_ref[...], wq_ref[...], preferred_element_type=jnp.float32)
            q_scr[...] = (q * scale).astype(jnp.bfloat16)

        row0 = pl.multiple_of(b * Sq, Sq)
        qb = q_scr[pl.ds(row0, Sq), :]
        qs = jnp.concatenate([qb[:, r * Dh:(r + 1) * Dh] for r in range(rep)], axis=0)
        k = k_ref[0, 0]
        v = v_ref[0, 0]
        s = lax.dot_general(qs, k, (((1,), (1,)), ((), ())),
                            preferred_element_type=jnp.float32)
        m = jnp.max(s, axis=-1, keepdims=True)
        p = jnp.exp(s - m)
        l = jnp.sum(p, axis=-1, keepdims=True)
        o = jnp.dot(p.astype(jnp.bfloat16), v, preferred_element_type=jnp.float32)
        o = (o / l).astype(jnp.bfloat16)
        ob = jnp.concatenate([o[r * Sq:(r + 1) * Sq, :] for r in range(rep)], axis=1)
        og_scr[pl.ds(row0, Sq), :] = ob

        @pl.when(b == B - 1)
        def _():
            contrib = jnp.dot(og_scr[...], wo_ref[...], preferred_element_type=jnp.float32)

            @pl.when(g == 0)
            def _():
                acc_scr[...] = contrib

            @pl.when(g > 0)
            def _():
                acc_scr[...] += contrib

            @pl.when(g == Hkv - 1)
            def _():
                o_ref[...] = acc_scr[...].astype(o_ref.dtype)

    out = pl.pallas_call(
        kernel,
        grid=(Hkv, B),
        in_specs=[
            pl.BlockSpec((M, D), lambda g, b: (0, 0)),
            pl.BlockSpec((D, GW), lambda g, b: (0, g)),
            pl.BlockSpec((1, 1, Sk, Dh), lambda g, b: (b, g, 0, 0)),
            pl.BlockSpec((1, 1, Sk, Dh), lambda g, b: (b, g, 0, 0)),
            pl.BlockSpec((GW, D), lambda g, b: (g, 0)),
        ],
        out_specs=pl.BlockSpec((M, D), lambda g, b: (0, 0)),
        out_shape=jax.ShapeDtypeStruct((M, D), x.dtype),
        scratch_shapes=[
            pltpu.VMEM((M, GW), jnp.bfloat16),
            pltpu.VMEM((M, GW), jnp.bfloat16),
            pltpu.VMEM((M, D), jnp.float32),
        ],
        compiler_params=pltpu.CompilerParams(
            dimension_semantics=("arbitrary", "arbitrary"),
            vmem_limit_bytes=96 * 1024 * 1024,
        ),
    )(x2, wq, k_cache, v_cache, wo)
    return out.reshape(B, Sq, D)
```

```python
import functools

import jax
import jax.numpy as jnp
from jax import lax
import jax.experimental.pallas as pl
import jax.experimental.pallas.tpu as pltpu

NSLOT = 8


@jax.jit
def pallas_standalone__gqa_block_cached__sampling_kernel(
    x: jax.Array,
    k_cache: jax.Array,
    v_cache: jax.Array,
    wq: jax.Array,
    wo: jax.Array,
):
    B, Sq, D = x.shape
    _, Hkv, Sk, Dh = k_cache.shape
    Hq = wq.shape[1] // Dh
    rep = Hq // Hkv
    M = B * Sq
    GW = rep * Dh
    NB = B * Hkv
    scale = float(Dh) ** -0.5

    x2 = x.reshape(M, D)

    def kernel(x_hbm, k_hbm, v_hbm, wq_hbm, wo_hbm, o_hbm,
               x_buf, wq_buf, wo_buf, kbuf, vbuf, q_scr, og_scr, acc_scr, out_scr,
               x_sem, wq_sem, wo_sem, k_sem, v_sem, out_sem):

        def kv_copies(i):
            slot = i % NSLOT
            g = i // B
            b = i % B
            return (pltpu.make_async_copy(k_hbm.at[b, g], kbuf.at[slot], k_sem.at[slot]),
                    pltpu.make_async_copy(v_hbm.at[b, g], vbuf.at[slot], v_sem.at[slot]))

        def wq_copy(g):
            return pltpu.make_async_copy(wq_hbm.at[:, pl.ds(g * GW, GW)], wq_buf.at[g], wq_sem.at[g])

        def wo_copy(g):
            return pltpu.make_async_copy(wo_hbm.at[pl.ds(g * GW, GW), :], wo_buf.at[g], wo_sem.at[g])

        x_copy = pltpu.make_async_copy(x_hbm, x_buf, x_sem)
        x_copy.start()
        wq_copy(0).start()
        for i in range(NSLOT):
            ck, cv = kv_copies(i)
            ck.start()
            cv.start()
        x_copy.wait()

        def body(i, carry):
            g = i // B
            b = i % B
            slot = i % NSLOT

            @pl.when(b == 0)
            def _():
                wo_copy(g).start()

                @pl.when(g + 1 < Hkv)
                def _():
                    wq_copy(g + 1).start()

                wq_copy(g).wait()
                q = jnp.dot(x_buf[...], wq_buf[g], preferred_element_type=jnp.float32)
                q_scr[...] = (q * scale).astype(jnp.bfloat16)

            ck, cv = kv_copies(i)
            ck.wait()
            cv.wait()

            row0 = pl.multiple_of(b * Sq, Sq)
            qb = q_scr[pl.ds(row0, Sq), :]
            qs = jnp.concatenate([qb[:, r * Dh:(r + 1) * Dh] for r in range(rep)], axis=0)
            k = kbuf[slot]
            v = vbuf[slot]
            s = lax.dot_general(qs, k, (((1,), (1,)), ((), ())),
                                preferred_element_type=jnp.float32)
            m = jnp.max(s, axis=-1, keepdims=True)
            p = jnp.exp(s - m)
            l = jnp.sum(p, axis=-1, keepdims=True)
            o = jnp.dot(p.astype(jnp.bfloat16), v, preferred_element_type=jnp.float32)
            o = (o / l).astype(jnp.bfloat16)
            ob = jnp.concatenate([o[r * Sq:(r + 1) * Sq, :] for r in range(rep)], axis=1)
            og_scr[pl.ds(row0, Sq), :] = ob

            @pl.when(i + NSLOT < NB)
            def _():
                nk, nv = kv_copies(i + NSLOT)
                nk.start()
                nv.start()

            @pl.when(b == B - 1)
            def _():
                wo_copy(g).wait()
                contrib = jnp.dot(og_scr[...], wo_buf[g], preferred_element_type=jnp.float32)

                @pl.when(g == 0)
                def _():
                    acc_scr[...] = contrib

                @pl.when(g > 0)
                def _():
                    acc_scr[...] += contrib

            return carry

        lax.fori_loop(0, NB, body, 0)
        out_scr[...] = acc_scr[...].astype(out_scr.dtype)
        oc = pltpu.make_async_copy(out_scr, o_hbm, out_sem)
        oc.start()
        oc.wait()

    out = pl.pallas_call(
        kernel,
        in_specs=[pl.BlockSpec(memory_space=pl.ANY)] * 5,
        out_specs=pl.BlockSpec(memory_space=pl.ANY),
        out_shape=jax.ShapeDtypeStruct((M, D), x.dtype),
        scratch_shapes=[
            pltpu.VMEM((M, D), x.dtype),
            pltpu.VMEM((Hkv, D, GW), wq.dtype),
            pltpu.VMEM((Hkv, GW, D), wo.dtype),
            pltpu.VMEM((NSLOT, Sk, Dh), k_cache.dtype),
            pltpu.VMEM((NSLOT, Sk, Dh), v_cache.dtype),
            pltpu.VMEM((M, GW), jnp.bfloat16),
            pltpu.VMEM((M, GW), jnp.bfloat16),
            pltpu.VMEM((M, D), jnp.float32),
            pltpu.VMEM((M, D), x.dtype),
            pltpu.SemaphoreType.DMA(()),
            pltpu.SemaphoreType.DMA((Hkv,)),
            pltpu.SemaphoreType.DMA((Hkv,)),
            pltpu.SemaphoreType.DMA((NSLOT,)),
            pltpu.SemaphoreType.DMA((NSLOT,)),
            pltpu.SemaphoreType.DMA(()),
        ],
        compiler_params=pltpu.CompilerParams(
            vmem_limit_bytes=100 * 1024 * 1024,
        ),
    )(x2, k_cache, v_cache, wq, wo)
    return out.reshape(B, Sq, D)
```

```python
import functools

import jax
import jax.numpy as jnp
from jax import lax
import jax.experimental.pallas as pl
import jax.experimental.pallas.tpu as pltpu

NSLOT = 8
CB = 4


@jax.jit
def pallas_standalone__gqa_block_cached__sampling_kernel(
    x: jax.Array,
    k_cache: jax.Array,
    v_cache: jax.Array,
    wq: jax.Array,
    wo: jax.Array,
):
    B, Sq, D = x.shape
    _, Hkv, Sk, Dh = k_cache.shape
    Hq = wq.shape[1] // Dh
    rep = Hq // Hkv
    M = B * Sq
    GW = rep * Dh
    NB = B * Hkv
    scale = float(Dh) ** -0.5

    x2 = x.reshape(M, D)

    def kernel(x_hbm, k_hbm, v_hbm, wq_hbm, wo_hbm, o_hbm,
               x_buf, wq_buf, wo_buf, kbuf, vbuf, q_scr, og_scr, acc_scr, out_scr,
               x_sem, wq_sem, wo_sem, k_sem, v_sem, out_sem):

        def kv_copies(i):
            slot = i % NSLOT
            g = i // B
            b = i % B
            return (pltpu.make_async_copy(k_hbm.at[b, g], kbuf.at[slot], k_sem.at[slot]),
                    pltpu.make_async_copy(v_hbm.at[b, g], vbuf.at[slot], v_sem.at[slot]))

        def wq_copy(g):
            return pltpu.make_async_copy(wq_hbm.at[:, pl.ds(g * GW, GW)], wq_buf.at[g], wq_sem.at[g])

        def wo_copy(g):
            return pltpu.make_async_copy(wo_hbm.at[pl.ds(g * GW, GW), :], wo_buf.at[g], wo_sem.at[g])

        x_copy = pltpu.make_async_copy(x_hbm, x_buf, x_sem)
        x_copy.start()
        wq_copy(0).start()
        for i in range(NSLOT):
            ck, cv = kv_copies(i)
            ck.start()
            cv.start()
        x_copy.wait()

        def body(i, carry):
            g = i // B
            b = i % B
            slot = i % NSLOT

            @pl.when(b == 0)
            def _():
                wo_copy(g).start()

                @pl.when(g + 1 < Hkv)
                def _():
                    wq_copy(g + 1).start()

                wq_copy(g).wait()
                q = jnp.dot(x_buf[...], wq_buf[g], preferred_element_type=jnp.float32)
                q_scr[...] = (q * scale).astype(jnp.bfloat16)

            ck, cv = kv_copies(i)
            ck.wait()
            cv.wait()

            row0 = pl.multiple_of(b * Sq, Sq)
            qb = q_scr[pl.ds(row0, Sq), :]
            qs = jnp.concatenate([qb[:, r * Dh:(r + 1) * Dh] for r in range(rep)], axis=0)
            k = kbuf[slot]
            v = vbuf[slot]
            s = lax.dot_general(qs, k, (((1,), (1,)), ((), ())),
                                preferred_element_type=jnp.float32)
            m = jnp.max(s, axis=-1, keepdims=True)
            p = jnp.exp(s - m)
            l = jnp.sum(p, axis=-1, keepdims=True)
            o = jnp.dot(p.astype(jnp.bfloat16), v, preferred_element_type=jnp.float32)
            o = (o / l).astype(jnp.bfloat16)
            ob = jnp.concatenate([o[r * Sq:(r + 1) * Sq, :] for r in range(rep)], axis=1)
            og_scr[pl.ds(row0, Sq), :] = ob

            @pl.when(i + NSLOT < NB)
            def _():
                nk, nv = kv_copies(i + NSLOT)
                nk.start()
                nv.start()

            @pl.when(b % CB == CB - 1)
            def _():
                @pl.when(b == CB - 1)
                def _():
                    wo_copy(g).wait()

                r0 = pl.multiple_of((b - (CB - 1)) * Sq, CB * Sq)
                rows = pl.ds(r0, CB * Sq)
                contrib = jnp.dot(og_scr[rows, :], wo_buf[g], preferred_element_type=jnp.float32)

                @pl.when(g == 0)
                def _():
                    acc_scr[rows, :] = contrib

                @pl.when(jnp.logical_and(g > 0, g < Hkv - 1))
                def _():
                    acc_scr[rows, :] += contrib

                @pl.when(g == Hkv - 1)
                def _():
                    out_scr[rows, :] = (acc_scr[rows, :] + contrib).astype(out_scr.dtype)
                    pltpu.make_async_copy(out_scr.at[rows, :], o_hbm.at[rows, :], out_sem.at[b // CB]).start()

            return carry

        lax.fori_loop(0, NB, body, 0)
        for c in range(B // CB):
            rows = pl.ds(c * CB * Sq, CB * Sq)
            pltpu.make_async_copy(out_scr.at[rows, :], o_hbm.at[rows, :], out_sem.at[c]).wait()

    out = pl.pallas_call(
        kernel,
        in_specs=[pl.BlockSpec(memory_space=pl.ANY)] * 5,
        out_specs=pl.BlockSpec(memory_space=pl.ANY),
        out_shape=jax.ShapeDtypeStruct((M, D), x.dtype),
        scratch_shapes=[
            pltpu.VMEM((M, D), x.dtype),
            pltpu.VMEM((Hkv, D, GW), wq.dtype),
            pltpu.VMEM((Hkv, GW, D), wo.dtype),
            pltpu.VMEM((NSLOT, Sk, Dh), k_cache.dtype),
            pltpu.VMEM((NSLOT, Sk, Dh), v_cache.dtype),
            pltpu.VMEM((M, GW), jnp.bfloat16),
            pltpu.VMEM((M, GW), jnp.bfloat16),
            pltpu.VMEM((M, D), jnp.float32),
            pltpu.VMEM((M, D), x.dtype),
            pltpu.SemaphoreType.DMA(()),
            pltpu.SemaphoreType.DMA((Hkv,)),
            pltpu.SemaphoreType.DMA((Hkv,)),
            pltpu.SemaphoreType.DMA((NSLOT,)),
            pltpu.SemaphoreType.DMA((NSLOT,)),
            pltpu.SemaphoreType.DMA((B // CB,)),
        ],
        compiler_params=pltpu.CompilerParams(
            vmem_limit_bytes=100 * 1024 * 1024,
        ),
    )(x2, k_cache, v_cache, wq, wo)
    return out.reshape(B, Sq, D)
```
